```python
import os as _os
_os.environ.setdefault("JAX_PLATFORMS", "cpu")
import jax
import jax.numpy as jnp

def _softmax(x, axis=-1):
    return jax.nn.softmax(x, axis=axis)
def _gelu(x):
    return jax.nn.gelu(x, approximate=True)
def _silu(x):
    return jax.nn.silu(x)
def _sigmoid(x):
    return jax.nn.sigmoid(x)
def _layernorm(x, axis=-1, eps=1e-5):
    m = jnp.mean(x, axis=axis, keepdims=True)
    v = jnp.var(x, axis=axis, keepdims=True)
    return (x - m) / jnp.sqrt(v + eps)
def _scatter_add(tgt, idx, src, axis=0):
    return tgt.at[idx].add(src)
def _segment_sum(src, seg, n):
    return jax.ops.segment_sum(src, seg, n)
class _Rng:
    def __init__(self, key):
        self._k = key
    def _next(self):
        self._k, sub = jax.random.split(self._k)
        return sub
    def normal(self, shape):
        return jax.random.normal(self._next(), shape, dtype=jnp.bfloat16)
    def randint(self, lo, hi, shape):
        return jax.random.randint(self._next(), shape, lo, hi, dtype=jnp.int32)
    def uniform(self, shape, lo=0.0, hi=1.0):
        return jax.random.uniform(self._next(), shape, jnp.bfloat16, lo, hi)
    def permutation(self, n):
        return jax.random.permutation(self._next(), n)


kernel_name = 'interleave_layers__sliding_local_dilated__mixer_s_mlp__prompt'

def setup_inputs():
    _rng = _Rng(jax.random.key(int.from_bytes(__import__("os").urandom(4), "little")))
    _w = (lambda a: (lambda t: t.astype(jnp.bfloat16) if jnp.issubdtype(t.dtype, jnp.floating) else t)(jnp.asarray(a)))
    def _A_setup():
        B, S, D = 1, 2048, 448
        return {
            "x": _w((lambda *s: _rng.normal(s) * 0.05)(B, S, D)),
            "wqkv": _w((lambda *s: _rng.normal(s) * 0.05)(D, 3 * D)),
            "wo": _w((lambda *s: _rng.normal(s) * 0.05)(D, D)),
        }
    _A_in = _A_setup()

    def _B_setup():
        B, S, D, F = 1, 2048, 448, 1792
        return {
            "x":  _w((lambda *s: _rng.normal(s) * 0.05)(B, S, D)),
            "w1": _w((lambda *s: _rng.normal(s) * 0.8)(D, D) * (D ** -0.5)),
            "w2": _w((lambda *s: _rng.normal(s) * 0.8)(D, D) * (D ** -0.5)),
            "w3": _w((lambda *s: _rng.normal(s) * 0.8)(D, F) * (D ** -0.5)),
            "w4": _w((lambda *s: _rng.normal(s) * 0.8)(F, D) * (F ** -0.5)),
        }
    _B_in = _B_setup()

    return {
        "A_x": _A_in["x"],
        "A_wqkv": _A_in["wqkv"],
        "A_wo": _A_in["wo"],
        "B_x": _B_in["x"],
        "B_w1": _B_in["w1"],
        "B_w2": _B_in["w2"],
        "B_w3": _B_in["w3"],
        "B_w4": _B_in["w4"],
    }

def reference(A_x, A_wqkv, A_wo, B_x, B_w1, B_w2, B_w3, B_w4):
    def _A_ref(x, wqkv, wo):
        B, S, D = x.shape
        H = 16; Dh = D // H
        W, dil = 8, 2
        qkv = (lambda x, *d: x.transpose(*d))((x @ wqkv).reshape(B, S, 3, H, Dh), 2, 0, 3, 1, 4)
        q, k, v = qkv[0], qkv[1], qkv[2]
        scale = Dh ** -0.5
        pos = jnp.arange(S)
        off = jnp.arange(W) * dil
        idx = pos[:, None] - off[None, :]
        mask = idx >= 0
        idx_c = jnp.where(mask, idx, 0).reshape(-1)
        kg = k[:, :, idx_c, :].reshape(B, H, S, W, Dh)
        vg = v[:, :, idx_c, :].reshape(B, H, S, W, Dh)
        logits = jnp.einsum("bhsd,bhswd->bhsw", q, kg) * scale
        logits = jnp.where(mask[None, None, :, :], logits, -1e9)
        attn = _softmax(logits, axis=-1)
        o = jnp.einsum("bhsw,bhswd->bhsd", attn, vg)
        return (lambda x, *d: x.transpose(*d))(o, 0, 2, 1, 3).reshape(B, S, D) @ wo

    def _B_ref(x, w1, w2, w3, w4):
        B, S, D = x.shape
        h = _gelu(_layernorm(x, axis=-1) @ w1)
        c = D // 4
        g0 = jnp.pad(h[:, :, 0*c:1*c], ((0, 0), (1, 0), (0, 0)))[:, :S, :]
        g1 = jnp.pad(h[:, :, 1*c:2*c], ((0, 0), (0, 1), (0, 0)))[:, 1:, :]
        g2 = jnp.pad(h[:, :, 2*c:3*c], ((0, 0), (2, 0), (0, 0)))[:, :S, :]
        g3 = jnp.pad(h[:, :, 3*c:   ], ((0, 0), (0, 2), (0, 0)))[:, 2:, :]
        hs = jnp.concatenate([g0, g1, g2, g3], axis=-1) @ w2
        x1 = x + hs
        h2 = _gelu(_layernorm(x1, axis=-1) @ w3) @ w4
        return x1 + h2

    x = A_x
    x = x + _A_ref(_layernorm(x, axis=-1), A_wqkv, A_wo)
    x = x + _B_ref(_layernorm(x, axis=-1), B_w1, B_w2, B_w3, B_w4)
    x = x + _A_ref(_layernorm(x, axis=-1), A_wqkv, A_wo)
    x = x + _B_ref(_layernorm(x, axis=-1), B_w1, B_w2, B_w3, B_w4)
    return x
```

```python
import functools
import math

import jax
import jax.numpy as jnp
import jax.experimental.pallas as pl
import jax.experimental.pallas.tpu as pltpu

S, D, F = 2048, 448, 1792
H, DH, W, DIL = 16, 28, 8, 2
T = 128
NT = S // T
NP = NT // 2
K1 = 256
EPS = 1e-5
f32, bf16, u32 = jnp.float32, jnp.bfloat16, jnp.uint32

_C0 = math.sqrt(2.0 / math.pi)
GA = (_C0 * 0.044715) ** (1.0 / 3.0)
GB = _C0 / GA

_HEAD = """s:x0 s:v s:k s:q s:x1 w:x0 N0 w:v p:v w:k s:wo s:w1 s:x2 v0 p:k w:q w:x1 s:w2 s:w3 s:w4
N1 p:q k0 q0 K0 N2 v1 k1 u2@P0/7@N2/5 q1 N3 P0 w:wo w:w1 w:x2 N4 u3@K1/7 K1 p:wo P1 p:w1 u4@P1/7 o0
w:w2 w:w3 w:w4 L0 K2 N5 o1 P2 a0@K2/6 L1 u5@P2/7 N6 K3 o2@N6/2 P3@u5 p:w2@u5 a1@p:w2/7@K3/6 G0 L2
u6@P3/7 N7 p:A@a1 p:B p:D@b0 b0@p:A/7 M0 p:C@a1 u7@p:B/2@p:C/4@p:D/7 o3 a2 L3 p:X@u7 p:Y@u7 p:Z@u7
a3 c0@p:X/1@p:Y/3 K4 G1 b1 P4 E0@P4/7 o4 M1"""
_STEP = "L4 c7 N0 K3@c7 a4@N0/5 G6@c7 u0@N0/1 P3@a4 E7@P3/1 b6 M6 o3@M6/6"
_TAIL = """L12 c9@L12/4 K13 a12@K13/6 G10@c9 P13@c9 E9@P13/7 b10@L12/5 M10 o13 L13 c10@L13/4 K14@c10 a13@L13/4
G11@c10 P14@c10 E10@P14/7 b11@L13/5 M11 o14 L14 c11@L14/4 K15@E10 a14 G12@c11 b12@L14/5 P15@E10
E11@P15/7 M12 o15 L15 c12@L15/6 a15 G13@c12 b13 E12 M13 c13 G14@c13 b14 E13 M14 G15@c14 b15 M15 c14
c15 E14 E15"""


def _program():
    head, tail = _HEAD.split(), _TAIL.split()
    done = [x.split("@")[0] for x in head + tail] + ["u0", "u1"]
    prog = list(head)
    for s in range(2 * NP + 7):
        for x in _STEP.split():
            parts = [y.partition("/") for y in x.split("@")]
            names = [t[0] + str(s - int(t[1:])) for t, _, _ in parts]
            if 0 <= s - int(parts[0][0][1:]) < 2 * NP and names[0] not in done:
                prog.append("@".join(n + c + k for n, (_, c, k) in zip(names, parts)))
    prog += tail
    prog.insert([x.split("@")[0] for x in prog].index("L13"), "|")
    return prog


def _ln(x):
    c = x - jnp.sum(x, axis=0, keepdims=True) * (1.0 / D)
    v = jnp.sum(c * c, axis=0, keepdims=True) * (1.0 / D)
    return c * jax.lax.rsqrt(v + EPS)


def _gelu(y):
    return y * jnp.tanh(y * (y * y + GB)) + y


def _dot(a, b):
    return jnp.dot(a, b.astype(bf16), preferred_element_type=f32)


def _padd(a, b, sign, axis):
    n = b.shape[axis]
    head = jax.lax.slice_in_dim(a, 0, n, axis=axis)
    head = head + b if sign > 0 else head - b
    if a.shape[axis] == n:
        return head
    return jnp.concatenate([head, jax.lax.slice_in_dim(a, n, a.shape[axis], axis=axis)], axis=axis)


def _left7(a11, a12, a21, a22, axis):
    short = jax.lax.slice_in_dim(a11, 0, a12.shape[axis], axis=axis)
    return (_padd(a11, a22, 1, axis), _padd(a21, a22, 1, axis), a11, a22, short + a12, a21 - a11, a12 - a22)


def _kernel(x_hbm, wqkv_hbm, wo_hbm, w1_hbm, w2_hbm, w3_hbm, w4_hbm, out_hbm,
            xin, wqkv_raw, wo_raw, w1_raw, w2_raw, w3_raw, w4_raw,
            wqkv7, wo7, w17, w27, w37, w47, tmps, bufs, outs, sem_in, sem_out):
    cols = lambda r, a, b: r.at[:, a:b]
    srcs = dict(
        x0=(cols(x_hbm, 0, 2 * T), cols(xin, 0, 2 * T)),
        x1=(cols(x_hbm, 2 * T, 8 * T), cols(xin, 2 * T, 8 * T)),
        x2=(cols(x_hbm, 8 * T, S), cols(xin, 8 * T, S)),
        q=(cols(wqkv_hbm, 0, 3 * T), cols(wqkv_raw, 0, 3 * T)),
        k=(cols(wqkv_hbm, 3 * T, 2 * D), cols(wqkv_raw, 3 * T, 2 * D)),
        v=(cols(wqkv_hbm, 2 * D, 3 * D), cols(wqkv_raw, 2 * D, 3 * D)),
        wo=(wo_hbm, wo_raw), w1=(w1_hbm, w1_raw), w2=(w2_hbm, w2_raw),
        w3=(w3_hbm, w3_raw), w4=(w4_hbm, w4_raw))
    copies = {n: pltpu.make_async_copy(a, b, sem_in.at[i]) for i, (n, (a, b)) in enumerate(srcs.items())}

    def out_copy(j):
        c = slice(j * T, (j + 1) * T)
        return pltpu.make_async_copy(outs.at[:, c], out_hbm.at[:, c], sem_out.at[j])

    def pin(i, carry):
        for r in jax.tree.leaves((bufs, tmps, wqkv7, wo7, w17, w27, w37, w47)):
            n = 16 if r.dtype == bf16 else 8
            row = pl.ds(pl.multiple_of(i * min(n, r.shape[-2] - n), n), n)
            r[(0,) * (len(r.shape) - 2) + (row, slice(0, T))] = jnp.zeros((n, T), r.dtype)
        return carry

    job, gates, signalled = {}, {}, []

    def signal(*vals):
        if job["name"] in gates:
            never = functools.reduce(jnp.logical_or, [jnp.abs(v[-8:]) < 0.0 for v in vals])
            gates[job["name"]][...] = jnp.where(never, 1.0, 0.0)
            signalled.append(job["name"])

    def zeros(at=0):
        return [gates[name] for name, n in job["after"] if name in signalled and n == at]

    def scaled(x, factor):
        for z in zeros():
            factor = factor + z[0:1, 0:x.shape[1]]
        return x * factor

    blocks = [(k0, min(T, D - k0)) for k0 in range(0, D, T)]
    w3v = w37.bitcast(bf16)

    def store7(dst, rows, kb, a11, a12, a21, a22):
        for i, a in enumerate(_left7(a11, a12, a21, a22, 1)):
            dst[i, kb, rows, 0:a.shape[1]] = a.astype(bf16)
            if a.shape[1] == T and isinstance(rows, slice):
                job["last"] = a

    def prep(dst, wt):
        for kb in range(2):
            t1, t2 = wt(kb), wt(kb + 2)
            m = t1.shape[0] // 2
            store7(dst, slice(0, m), kb, t1[:m], t2[:m], t1[m:], t2[m:])

    def prep_plain(src, dst, factor):
        prep(dst, lambda kb: scaled(src[blocks[kb][0]:sum(blocks[kb]), :].T.astype(f32), factor))

    def prep_qkv(p, rolled):
        n0 = p * D // T * T
        tmp = tmps[p % 2]
        for kb, (k0, kw) in enumerate(blocks):
            for c0 in range(n0, (p + 1) * D, T):
                cw = min(T, 3 * D - c0)
                tmp[kb, c0 - n0:c0 - n0 + cw, 0:kw] = wqkv_raw[k0:k0 + kw, c0:c0 + cw].T.astype(f32)
        blk = lambda kb, d: tmp[kb, pl.ds(p * D - n0 + d, H, stride=DH), :][:, 0:blocks[kb][1]]

        def group(d, carry):
            r0 = p * D // 2 + d * H
            rows = pl.ds(pl.multiple_of(r0, H) if rolled else r0, H)
            for kb in range(2):
                store7(wqkv7, rows, kb, blk(kb, d), blk(kb + 2, d), blk(kb, d + DH // 2), blk(kb + 2, d + DH // 2))
            return carry
        if rolled:
            jax.lax.fori_loop(0, DH // 2, group, 0)
        else:
            for d in range(DH // 2):
                group(d, 0)

    def prep_wo():
        tmp = tmps[0]
        for nb, (n0, nw) in enumerate(blocks):
            tmp[nb, 0:D, 0:nw] = wo_raw[:, n0:n0 + nw].astype(f32)

        def wt(kb):
            ds = range(blocks[kb][0] // H, sum(blocks[kb]) // H)
            return jnp.concatenate([
                jnp.concatenate([tmp[nb, pl.ds(d, H, stride=DH), :] for d in ds], axis=0)[:, 0:nw]
                .astype(bf16).T.astype(f32) for nb, (_, nw) in enumerate(blocks)], axis=0)
        prep(wo7, wt)

    def prep_w3(kb, n0, n1):
        (ka, wa), (kc, wc) = blocks[kb], blocks[kb + 2]
        for c0 in range(n0 * T, n1 * T, T):
            get = lambda k0, kw, c: scaled(w3_raw[k0:k0 + kw, c:c + T].astype(f32), GA)
            for i, a in enumerate(_left7(get(ka, wa, c0), get(kc, wc, c0), get(ka, wa, F // 2 + c0),
                                         get(kc, wc, F // 2 + c0), 0)):
                y = a.astype(bf16).T
                w3v[i, c0:c0 + T, kb * T:kb * T + a.shape[0]] = y
                if a.shape[0] == T:
                    job["last"] = y[0:H].astype(f32)

    def prep_w4(r0, r1):
        get = lambda r, c: scaled(w4_raw[r:r + H, c:c + T].astype(f32), 0.5 / GA)
        for r in range(r0, r1, H):
            for c in range(0, F // 2, T):
                store7(w47, slice(r, r + H), c // T, get(r, c), get(r, F // 2 + c),
                       get(D // 2 + r, c), get(D // 2 + r, F // 2 + c))

    preps = dict(
        q=lambda: prep_qkv(0, False), k=lambda: prep_qkv(1, False), v=lambda: prep_qkv(2, True), wo=prep_wo,
        w1=lambda: prep_plain(w1_raw, w17, GA), w2=lambda: prep_plain(w2_raw, w27, 0.5 / GA),
        A=lambda: prep_w3(0, 0, 4), B=lambda: prep_w3(0, 4, 7), C=lambda: prep_w3(1, 0, 4), D=lambda: prep_w3(1, 4, 7),
        X=lambda: prep_w4(0, 80), Y=lambda: prep_w4(80, 160), Z=lambda: prep_w4(160, D // 2))

    def buf(name, u):
        return bufs[name][u % len(bufs[name])]

    def get_x(u, i, rows=slice(0, D)):
        if u < NP:
            return xin[rows, (2 * u + i) * T:(2 * u + i + 1) * T].astype(f32)
        return buf("x", u)[i, rows, :]

    count = [0]

    def strassen(w, src, k1, emit, rows=None):
        k = src.shape[1]
        r0, r1 = rows or (0, w.shape[-2])
        b11 = lambda n=k1: src[0, 0:n, :]
        b21 = lambda: src[0, k1:k, :]
        b12 = lambda: src[1, 0:k1, :]
        b22 = lambda: src[1, k1:k, :]
        right = (lambda: _padd(b11(), b22(), 1, 0), b11, lambda: _padd(b12(), b22(), -1, 0),
                 lambda: b21() - b11(k - k1), b22, lambda: b11() + b12(), lambda: b21() + b22())

        def left(i, a, b, c0, c1):
            if len(w.shape) == 3:
                return w[i - 1, a:b, c0:c1]
            w32 = w.bitcast(u32)
            return jnp.concatenate([pltpu.bitcast(w32[i - 1, c // T, a // 2:b // 2, 0:min(T, c1 - c)], bf16)
                                    for c in range(c0, c1, T)], axis=1)

        def prod(i):
            b = right[i - 1]()
            for z in zeros(1 + (1, 4, 5, 7, 6, 2, 3).index(i)):
                b = jnp.concatenate([b[0:8] + z[...], b[8:]], axis=0)
            n = b.shape[0]
            if n == F // 2 and i == 3:
                m = (r0 + r1) // 2
                return _dot(left(i, r0, r1, 0, n - T), b[0:n - T]) + jnp.concatenate(
                    [_dot(left(i, a, c, n - T, n), b[n - T:n]) for a, c in ((r0, m), (m, r1))], axis=0)
            return _dot(left(i, r0, r1, 0, n), b)

        count[0] += 1
        s1, s4, s5, s6 = [part.at[0:r1 - r0, :] for part in bufs["part"]]
        s1[...] = prod(1)
        s4[...] = prod(4)
        s5[...] = prod(5)
        emit(0, 0, ((prod(7) + s1[...]) + s4[...]) - s5[...])
        m6 = prod(6)
        m2 = prod(2)
        emit(0, 1, m2 + s4[...])
        together = count[0] % 2 == 0
        s6[...] = (m6 if together else m6 - m2) + s1[...]
        m3 = prod(3)
        emit(1, 0, m3 + s5[...])
        c22 = ((m3 - m2) if together else m3) + s6[...]
        signal(c22)
        emit(1, 1, c22)

    def half(h, n=D):
        return slice(h * (n // 2), (h + 1) * (n // 2))

    def norm(dst, get):
        ys = [_ln(get(i)) for i in range(2)]
        for i in range(2):
            dst[i] = ys[i]
        return ys

    def project(u, p0, p1):
        m = D // 2

        def emit(i, h, val):
            for n, p in enumerate(range(p0, p1)):
                buf("qkv"[p], u)[i, half(h), :] = val[n * m:(n + 1) * m]
        strassen(wqkv7, buf("xn", u), K1, emit, (p0 * m, p1 * m))

    def window(name, t, d, lane):
        rows = slice(d * H, (d + 1) * H)
        cur = buf(name, t // 2)[t % 2, rows, :]
        if t % NT:
            prev = buf(name, (t - 1) // 2)[(t - 1) % 2, rows, :]
        else:
            prev = jnp.broadcast_to(cur[:, 0:1], (H, T)) if name == "v" else cur
        return [cur] + [pltpu.roll(jnp.where(lane >= T - DIL * w, prev, cur), DIL * w, 1) for w in range(1, W)]

    def lanes():
        lane = jax.lax.broadcasted_iota(jnp.int32, (H, T), 1)
        for z in zeros():
            lane = lane + z[0:1, :].astype(jnp.int32)
        return lane

    def probs(u):
        lane, rs = lanes(), []
        for i in range(2):
            for d in range(DH):
                q = buf("q", u)[i, d * H:(d + 1) * H, :]
                prs = [q * k for k in window("k", 2 * u + i, d, lane)]
                acc = prs if d == 0 else [a + b for a, b in zip(acc, prs)]
            lg = [a * (DH ** -0.5) for a in acc]
            if (2 * u + i) % NT == 0:
                lg = [lg[0]] + [jnp.where(lane >= DIL * w, lg[w], -1e9) for w in range(1, W)]
            mx = functools.reduce(jnp.maximum, lg)
            e = [jnp.exp(x - mx) for x in lg]
            rs.append(1.0 / functools.reduce(lambda a, b: a + b, e))
            for w in range(W):
                buf("p", u)[i, w * H:(w + 1) * H, :] = e[w] * rs[-1]
        signal(*rs)

    def mix(u):
        lane, last = lanes(), []
        for i in range(2):
            for d in range(DH):
                prs = [buf("p", u)[i, w * H:(w + 1) * H, :] * v for w, v in enumerate(window("v", 2 * u + i, d, lane))]
                while len(prs) > 1:
                    prs = [a + b for a, b in zip(prs[0::2], prs[1::2])]
                buf("o", u)[i, d * H:(d + 1) * H, :] = prs[0]
            last.append(prs[0])
        signal(*last)

    def mm_o(u):
        def emit(i, h, val):
            buf("x1", u)[i, half(h), :] = get_x(u, i, half(h)) + val
        strassen(wo7, buf("o", u), K1, emit)

    def norms(u):
        norm(buf("xb", u), lambda i: buf("x1", u)[i])
        signal(*norm(buf("xbn", u), lambda i: buf("xb", u)[i]))

    def mm_1(u):
        def emit(i, h, val):
            buf("h", u)[i, half(h), :] = _gelu(val)
        strassen(w17, buf("xbn", u), K1, emit)

    def shift(u):
        c = D // 4
        lane = jax.lax.broadcasted_iota(jnp.int32, (c, T), 1)
        for t in (2 * u, 2 * u + 1):
            for n, sh in enumerate((1, -1, 2, -2)):
                rows, nb = slice(n * c, (n + 1) * c), -1 if sh > 0 else 1
                cur = buf("h", u)[t % 2, rows, :]
                other = jnp.zeros_like(cur)
                if 0 <= t % NT + nb < NT:
                    other = buf("h", (t + nb) // 2)[(t + nb) % 2, rows, :]
                edge = (lane >= T - sh) if sh > 0 else (lane < -sh)
                buf("g", u)[t % 2, rows, :] = pltpu.roll(jnp.where(edge, other, cur), sh % T, 1)

    def mm_2(u):
        def emit(i, h, val):
            buf("x1b", u)[i, half(h), :] = buf("xb", u)[i, half(h), :] + val
        strassen(w27, buf("g", u), K1, emit)

    def mm_3(u):
        def emit(i, h, val):
            buf("h2", u)[i, half(h, F), :] = _gelu(val)
        strassen(w3v, buf("xcn", u), K1, emit)

    def mm_4(u):
        def emit(i, h, val):
            y = buf("x1", u)[i, half(h), :] + (buf("x1b", u)[i, half(h), :] + val)
            if u < NP:
                buf("x", u)[i, half(h), :] = y
            else:
                j = 2 * (u - NP) + i
                outs[half(h), j * T:(j + 1) * T] = y.astype(bf16)
                if h == 1:
                    out_copy(j).start()
        strassen(w47, buf("h2", u), F // 2, emit)

    jobs = dict(
        N=lambda u: signal(*norm(buf("xn", u), lambda i: get_x(u, i))),
        u=lambda u: project(u, 0, 3), q=lambda u: project(u, 0, 1), k=lambda u: project(u, 1, 2),
        v=lambda u: project(u, 2, 3), K=probs, P=mix, o=mm_o, L=norms, a=mm_1, G=shift, b=mm_2,
        M=lambda u: signal(*norm(buf("xcn", u), lambda i: buf("x1b", u)[i])), c=mm_3, E=mm_4)

    prog = _program()
    names = [x.split("@")[0] for x in prog]
    for n, x in enumerate(prog):
        for r in x.split("@")[1:]:
            r = r.partition("/")[0]
            if r in names[:n] and r not in gates:
                gates[r] = buf("gate", len(gates))
    for n, x in enumerate(prog):
        name, *after = x.split("@")
        job.clear()
        job.update(name=name, after=[(r.partition("/")[0], int(r.partition("/")[2] or 0)) for r in after])
        if name == "w:x0":
            jax.lax.fori_loop(0, 2, pin, 0)
        if name == "|":
            out_copy(0).wait()
        elif name.startswith("s:"):
            copies[name[2:]].start()
        elif name.startswith("w:"):
            copies[name[2:]].wait()
        elif name.startswith("p:"):
            preps[name[2:]]()
            if "last" in job:
                signal(job["last"])
        else:
            jobs[name[0]](int(name[1:]))
    for j in range(1, NT):
        out_copy(j).wait()


@jax.jit
def pallas_interleave_layers__sliding_local_dilated__mixer_s_mlp__prompt_kernel(
    A_x: jax.Array,
    A_wqkv: jax.Array,
    A_wo: jax.Array,
    B_x: jax.Array,
    B_w1: jax.Array,
    B_w2: jax.Array,
    B_w3: jax.Array,
    B_w4: jax.Array,
):
    del B_x
    V = pltpu.VMEM
    pairs = dict(x=NP, x1=7, xb=4, x1b=4, q=5, k=5, v=5, h=5, xn=2, o=2, xbn=2, g=2, xcn=2)
    bufs = {n: [V((2, D, T), f32)] * k for n, k in pairs.items()}
    bufs.update(h2=[V((2, F, T), f32)] * 2, p=[V((2, W * H, T), f32)] * 2,
                part=[V((F // 2, T), f32)] * 4, gate=[V((8, T), f32)] * 16)
    out = pl.pallas_call(
        _kernel,
        out_shape=jax.ShapeDtypeStruct((D, S), bf16),
        in_specs=[pl.BlockSpec(memory_space=pl.ANY)] * 7,
        out_specs=pl.BlockSpec(memory_space=pl.ANY),
        scratch_shapes=[
            V((D, S), bf16), V((D, 3 * D), bf16), V((D, D), bf16), V((D, D), bf16), V((D, D), bf16),
            V((D, F), bf16), V((D, F), bf16),
            V((7, 2, 3 * D // 2, T), bf16), V((7, 2, D // 2, T), bf16), V((7, 2, D // 2, T), bf16),
            V((7, 2, D // 2, T), bf16), V((7, F // 4, K1), u32), V((7, F // 2 // T, D // 2, T), bf16),
            [V((4, 5 * T, T), f32)] * 2, bufs, V((D, S), bf16),
            pltpu.SemaphoreType.DMA((11,)), pltpu.SemaphoreType.DMA((NT,)),
        ],
        compiler_params=pltpu.CompilerParams(
            vmem_limit_bytes=100 * 1024 * 1024,
            flags={"XLA_TPU_FORCE_LP_LLO_SCHEDULER": True}),
    )(A_x.reshape(S, D).T, A_wqkv, A_wo, B_w1, B_w2, B_w3, B_w4.T)
    return out.T.reshape(1, S, D)
```
